```python
import os as _os
_os.environ.setdefault("JAX_PLATFORMS", "cpu")
import jax
import jax.numpy as jnp

def _softmax(x, axis=-1):
    return jax.nn.softmax(x, axis=axis)
def _gelu(x):
    return jax.nn.gelu(x, approximate=True)
def _silu(x):
    return jax.nn.silu(x)
def _sigmoid(x):
    return jax.nn.sigmoid(x)
def _layernorm(x, axis=-1, eps=1e-5):
    m = jnp.mean(x, axis=axis, keepdims=True)
    v = jnp.var(x, axis=axis, keepdims=True)
    return (x - m) / jnp.sqrt(v + eps)
def _scatter_add(tgt, idx, src, axis=0):
    return tgt.at[idx].add(src)
def _segment_sum(src, seg, n):
    return jax.ops.segment_sum(src, seg, n)
class _Rng:
    def __init__(self, key):
        self._k = key
    def _next(self):
        self._k, sub = jax.random.split(self._k)
        return sub
    def normal(self, shape):
        return jax.random.normal(self._next(), shape, dtype=jnp.bfloat16)
    def randint(self, lo, hi, shape):
        return jax.random.randint(self._next(), shape, lo, hi, dtype=jnp.int32)
    def uniform(self, shape, lo=0.0, hi=1.0):
        return jax.random.uniform(self._next(), shape, jnp.bfloat16, lo, hi)
    def permutation(self, n):
        return jax.random.permutation(self._next(), n)


kernel_name = 'interleave_layers__sliding_block__dense_activation_gelu__prompt'

def setup_inputs():
    _rng = _Rng(jax.random.key(int.from_bytes(__import__("os").urandom(4), "little")))
    _w = (lambda a: (lambda t: t.astype(jnp.bfloat16) if jnp.issubdtype(t.dtype, jnp.floating) else t)(jnp.asarray(a)))
    def _A_setup():
        B, S, D = 1, 2048, 640
        return {
            "x": _w((lambda *s: _rng.normal(s) * 0.05)(B, S, D)),
            "wqkv": _w((lambda *s: _rng.normal(s) * 0.05)(D, 3 * D)),
            "wo": _w((lambda *s: _rng.normal(s) * 0.05)(D, D)),
        }
    _A_in = _A_setup()

    def _B_setup():
        B, S, D, F = 1, 2048, 640, 1728
        return {
            "x": _w((lambda *s: _rng.normal(s) * 0.05)(B, S, D)),
            "w1": _w((lambda *s: _rng.normal(s) * 0.8)(D, F) * (D ** -0.5)),
            "b1": _w((lambda *s: _rng.normal(s) * 0.8)(F) * 0.01),
            "w2": _w((lambda *s: _rng.normal(s) * 0.8)(F, D) * (F ** -0.5)),
            "b2": _w((lambda *s: _rng.normal(s) * 0.8)(D) * 0.01),
        }
    _B_in = _B_setup()

    return {
        "A_x": _A_in["x"],
        "A_wqkv": _A_in["wqkv"],
        "A_wo": _A_in["wo"],
        "B_x": _B_in["x"],
        "B_w1": _B_in["w1"],
        "B_b1": _B_in["b1"],
        "B_w2": _B_in["w2"],
        "B_b2": _B_in["b2"],
    }

def reference(A_x, A_wqkv, A_wo, B_x, B_w1, B_b1, B_w2, B_b2):
    def _A_ref(x, wqkv, wo):
        B, S, D = x.shape
        H = 32; Dh = D // H; W = 256
        qkv = (lambda x, *d: x.transpose(*d))((x @ wqkv).reshape(B, S, 3, H, Dh), 2, 0, 3, 1, 4)
        q, k, v = qkv[0], qkv[1], qkv[2]
        scores = jnp.einsum("bhqd,bhkd->bhqk", q, k) * (Dh ** -0.5)
        idx = jnp.arange(S)
        mask = (idx[:, None] - idx[None, :] >= 0) & (idx[:, None] - idx[None, :] < W)
        scores = jnp.where(mask[None, None], scores, -1e9)
        p = _softmax(scores, axis=-1)
        o = jnp.einsum("bhqk,bhkd->bhqd", p, v)
        return (lambda x, *d: x.transpose(*d))(o, 0, 2, 1, 3).reshape(B, S, D) @ wo

    def _B_ref(x, w1, b1, w2, b2):
        h = jnp.einsum("bsd,df->bsf", x, w1) + b1
        h = _gelu(h)
        return jnp.einsum("bsf,fd->bsd", h, w2) + b2

    x = A_x
    x = x + _A_ref(_layernorm(x, axis=-1), A_wqkv, A_wo)
    x = x + _B_ref(_layernorm(x, axis=-1), B_w1, B_b1, B_w2, B_b2)
    x = x + _A_ref(_layernorm(x, axis=-1), A_wqkv, A_wo)
    x = x + _B_ref(_layernorm(x, axis=-1), B_w1, B_b1, B_w2, B_b2)
    return x
```

```python
import math
import jax
import jax.numpy as jnp
from jax import lax
import jax.experimental.pallas as pl
import jax.experimental.pallas.tpu as pltpu

S, D, H, DH, W, F = 2048, 640, 32, 20, 256, 1728
G = 8
QB = 32
KW = W + QB
BM = 512
NEG = -1e30
QSCALE = (DH ** -0.5) * math.log2(math.e)
G_TILE = (0, 5, 1, 6, 7, 3, 8, 4)
G_OFF = (0, 16, 32, 48, 0, 16, 32, 48)


def _pk(v):
    return pltpu.bitcast(v, jnp.uint32)


def _up(v):
    return pltpu.bitcast(v, jnp.bfloat16)


def _ln(x):
    m = jnp.mean(x, axis=-1, keepdims=True)
    xc = x - m
    v = jnp.mean(xc * xc, axis=-1, keepdims=True)
    return xc * lax.rsqrt(v + 1e-5)


def _kernel(x_hbm, wqkv_hbm, wo_hbm, w1_hbm, b1_ref, w2_hbm, b2_ref, out_hbm,
            x_ref, wqkv_ref, wo_ref, w1_ref, w2_ref, obuf, sems,
            xres, qs, ks, vt, ot, wvt, sb0, sb1, pb0, pb1):
    sb = (sb0, sb1)
    pb = (pb0, pb1)
    f32, bf16, u32 = jnp.float32, jnp.bfloat16, jnp.uint32
    NC = S // BM
    x_cp = [pltpu.make_async_copy(x_hbm.at[pl.ds(c_ * BM, BM)], x_ref.at[pl.ds(c_ * BM, BM)], sems.at[c_])
            for c_ in range(NC)]
    w_cp = [pltpu.make_async_copy(h_, v_, sems.at[NC + i_]) for i_, (h_, v_) in enumerate(
        ((wqkv_hbm, wqkv_ref), (wo_hbm, wo_ref), (w1_hbm, w1_ref), (w2_hbm, w2_ref)))]
    w_cp[0].start()
    for cp in x_cp:
        cp.start()
    for cp in w_cp[1:]:
        cp.start()
    qs_b, ks_b, vt_b, ot_b, pb_b = qs, ks, vt, ot, pb
    qs, ks, vt, ot = [r.bitcast(u32) for r in (qs, ks, vt, ot)]
    pb = [r.bitcast(u32) for r in pb]
    vt[0:2] = jnp.zeros((2, G, 48, 128), u32)
    for r_ in pb:
        r_[...] = jnp.zeros((4, 192, 128), u32)
    ones_rows = jnp.where(lax.broadcasted_iota(jnp.int32, (16, 128), 0) < 8, 1.0, 0.0).astype(bf16)
    for t_ in range(2, 18):
        if True:
            vt[t_, :, 40:48] = jnp.broadcast_to(_pk(ones_rows), (G, 8, 128))

    w_cp[0].wait()
    wvt[...] = wqkv_ref[:, 2 * D:].astype(f32).T.astype(bf16)
    for cp in x_cp:
        cp.wait()

    def out_copy(c):
        return pltpu.make_async_copy(obuf.at[pl.ds(c * BM, BM)], out_hbm.at[pl.ds(c * BM, BM)], sems.at[NC + 4])

    def qkv_chunk(c, first):
        r0 = pl.multiple_of(c * BM, BM)
        if first:
            xc = x_ref[pl.ds(r0, BM), :].astype(f32)
            xres[pl.ds(r0, BM), :] = xc
        else:
            xc = xres[pl.ds(r0, BM), :]
        xb = _ln(xc).astype(bf16)
        q = (jnp.dot(xb, wqkv_ref[:, 0:D], preferred_element_type=f32) * QSCALE).astype(bf16)
        k = jnp.dot(xb, wqkv_ref[:, D:2 * D], preferred_element_type=f32).astype(bf16)
        rh = pl.multiple_of(c * (BM // 2), BM // 2)
        lo64 = lax.broadcasted_iota(jnp.int32, (BM // 2, 128), 1) < 64
        for val, refb, ref, base in ((q, qs_b, qs, 0), (k, ks_b, ks, W)):
            for t in range(5):
                refb[t, pl.ds(base + r0, BM), :] = val[:, 128 * t:128 * (t + 1)]
            rl = [pltpu.roll(ref[t, pl.ds(base // 2 + rh, BM // 2), :], 64, 1) for t in range(5)]
            for t in range(4):
                ref[5 + t, pl.ds(base // 2 + rh, BM // 2), :] = jnp.where(lo64, rl[t], rl[t + 1])
        vT = lax.dot_general(wvt[...], xb, (((1,), (1,)), ((), ())),
                             preferred_element_type=f32).astype(bf16)
        nt = BM // 128
        for t in range(nt):
            for g in range(G):
                vt_b[2 + c * nt + t, g, 0:80] = vT[80 * g:80 * (g + 1), 128 * t:128 * (t + 1)]

    lane = lax.broadcasted_iota(jnp.int32, (128, 128), 1)
    row = lax.broadcasted_iota(jnp.int32, (128, 128), 0)
    r32 = lax.broadcasted_iota(jnp.int32, (QB, 128), 0)
    c32 = lax.broadcasted_iota(jnp.int32, (QB, 128), 1) % QB
    orow = lax.broadcasted_iota(jnp.int32, (80, 128), 0) // DH
    olane = lax.broadcasted_iota(jnp.int32, (80, 128), 1) // QB

    r8 = lax.broadcasted_iota(jnp.int32, (8, 128), 0)
    l8 = lax.broadcasted_iota(jnp.int32, (8, 128), 1) // QB

    def stage_a(g, J, s, sref):
        tile = jnp.int32(0)
        off = jnp.int32(0)
        for gg in range(G):
            tile = jnp.where(g == gg, G_TILE[gg], tile)
            off = jnp.where(g == gg, G_OFF[gg], off)
        lo = off + DH * (row // QB)
        qmask = (lane >= lo) & (lane < lo + DH)
        qh = pl.multiple_of(J * 64 + s * (QB // 2), QB // 2)
        q = _up(qs[tile, pl.ds(qh, QB // 2), :])
        qbd = jnp.where(qmask, jnp.concatenate([q] * 4, axis=0), jnp.zeros((), bf16))
        kb = _up(ks[tile, pl.ds(qh, KW // 2), :])
        sref[...] = lax.dot_general(kb, qbd, (((1,), (1,)), ((), ())), preferred_element_type=f32)

    def stage_b(sref, pref):
        po = QB * pref[0]
        pref = pref[1].at[pref[0]]
        top = jnp.where(r32 > c32, sref[0:QB], NEG)
        bot = jnp.where(r32 <= c32, sref[W:KW], NEG)
        mid = [sref[QB + 32 * i:QB + 32 * (i + 1)] for i in range(7)]
        parts = [top] + mid + [bot]
        mx = parts[0]
        for t in parts[1:]:
            mx = jnp.maximum(mx, t)
        m = jnp.max(mx, axis=0, keepdims=True)
        for i, t in enumerate(parts):
            pref[po + 32 * i:po + 32 * (i + 1)] = jnp.exp2(t - m).astype(bf16)

    def stage_c(g, J, s, pref, acc):
        o = jnp.dot(_up(vt[J, g]), _up(pref[0:64]), preferred_element_type=f32)
        o += jnp.dot(_up(vt[J + 1, g]), _up(pref[64:128]), preferred_element_type=f32)
        o += jnp.dot(_up(vt[J + 2, g]), _up(pref[128:192]), preferred_element_type=f32)
        rl = 1.0 / o[80:88]
        for i in range(10):
            oi = o[8 * i:8 * i + 8] * rl
            for h in sorted({(8 * i) // DH, (8 * i + 7) // DH}):
                sh = (QB * (s - h)) % 128
                oo = oi if sh == 0 else pltpu.roll(oi, sh, 1)
                msk = l8 == s
                if (8 * i) // DH != (8 * i + 7) // DH:
                    msk = msk & ((r8 + 8 * i) // DH == h)
                acc[i] = jnp.where(msk, oo, acc[i])

    def store_o(g, J, acc):
        ot_b[J, pl.ds(pl.multiple_of(g * 80, 16), 80), :] = jnp.concatenate(acc, axis=0).astype(bf16)

    NF = S // 128

    def gj(i):
        i = jnp.minimum(i, G * NF - 1)
        return i // NF, i % NF

    def a_fast(i2, _):
        for par in range(2):
            i = 2 * i2 + par
            g, J = gj(i)
            g2, J2 = gj(i + 2)
            acc = [jnp.zeros((8, 128), f32)] * 10
            for s in range(4):
                stage_b(sb[1 - par].at[s], (s, pb_b[1 - par]))
            for s in range(4):
                stage_c(g, J, s, pb[par].at[s], acc)
            for s in range(4):
                stage_a(g2, J2, s, sb[par].at[s])
            store_o(g, J, acc)
        return 0

    def post_chunk(c, last):
        r0 = pl.multiple_of(c * BM, BM)
        nt = BM // 128
        oT = jnp.concatenate([_up(ot[c * nt + t]) for t in range(nt)], axis=1)
        a = lax.dot_general(oT, wo_ref[...], (((0,), (0,)), ((), ())), preferred_element_type=f32)
        x1 = xres[pl.ds(r0, BM), :] + a
        xb = _ln(x1).astype(bf16)
        hpre = lax.dot_general(xb, w1_ref[...], (((1,), (1,)), ((), ())), preferred_element_type=f32) + b1_ref[...].astype(f32).reshape(1, F)
        hh = jax.nn.gelu(hpre, approximate=True).astype(bf16)
        y = jnp.dot(hh, w2_ref[...], preferred_element_type=f32) + b2_ref[...].astype(f32).reshape(1, D)
        x2 = x1 + y
        if last:
            obuf[pl.ds(r0, BM), :] = x2.astype(obuf.dtype)
            out_copy(c).start()
        else:
            xres[pl.ds(r0, BM), :] = x2

    for layer in range(2):
        def qkv_body(c, _, first=(layer == 0)):
            qkv_chunk(c, first)
            return 0
        with jax.named_scope("qkv"):
            with jax.named_scope("a"):
                lax.fori_loop(0, S // BM, qkv_body, 0)

        with jax.named_scope("attn"):
            for t_ in range(9):
                ks_b[t_, 0:W, :] = jnp.broadcast_to(ks_b[t_, W:W + 16, :][0:1], (W, 128))
            for s_ in range(4):
                stage_a(jnp.int32(0), jnp.int32(0), s_, sb[0].at[s_])
            for s_ in range(4):
                stage_a(jnp.int32(0), jnp.int32(1), s_, sb[1].at[s_])
            for s_ in range(4):
                stage_b(sb[0].at[s_], (s_, pb_b[0]))
            lax.fori_loop(0, G * NF // 2, a_fast, 0)

        if layer == 0:
            for cp in w_cp[1:]:
                cp.wait()

        def post_body(c, _, last=(layer == 1)):
            post_chunk(c, last)
            return 0
        with jax.named_scope("post"):
            lax.fori_loop(0, S // BM, post_body, 0)
    for c_ in range(NC):
        out_copy(c_).wait()


@jax.jit
def pallas_interleave_layers__sliding_block__dense_activation_gelu__prompt_kernel(
        A_x, A_wqkv, A_wo, B_x, B_w1, B_b1, B_w2, B_b2):
    del B_x
    bf16 = jnp.bfloat16
    out = pl.pallas_call(
        _kernel,
        out_shape=jax.ShapeDtypeStruct((S, D), A_x.dtype),
        in_specs=[pl.BlockSpec(memory_space=pl.ANY)] * 4 + [pl.BlockSpec(memory_space=pltpu.VMEM),
                                                             pl.BlockSpec(memory_space=pl.ANY),
                                                             pl.BlockSpec(memory_space=pltpu.VMEM)],
        out_specs=pl.BlockSpec(memory_space=pl.ANY),
        scratch_shapes=[
            pltpu.VMEM((S, D), bf16),
            pltpu.VMEM((D, 3 * D), bf16),
            pltpu.VMEM((D, D), bf16),
            pltpu.VMEM((F, D), bf16),
            pltpu.VMEM((F, D), bf16),
            pltpu.VMEM((S, D), bf16),
            pltpu.SemaphoreType.DMA((S // BM + 5,)),
            pltpu.VMEM((S, D), jnp.float32),
            pltpu.VMEM((9, S, 128), bf16),
            pltpu.VMEM((9, S + W, 128), bf16),
            pltpu.VMEM((18, G, 96, 128), bf16),
            pltpu.VMEM((16, D, 128), bf16),
            pltpu.VMEM((D, D), bf16),
            pltpu.VMEM((4, KW, 128), jnp.float32),
            pltpu.VMEM((4, KW, 128), jnp.float32),
            pltpu.VMEM((4, 384, 128), bf16),
            pltpu.VMEM((4, 384, 128), bf16),
        ],
        compiler_params=pltpu.CompilerParams(vmem_limit_bytes=100 * 1024 * 1024),
    )(A_x.reshape(S, D), A_wqkv, A_wo, B_w1.T, B_b1, B_w2, B_b2)
    return out.reshape(1, S, D)
```

```python
import math
import jax
import jax.numpy as jnp
from jax import lax
import jax.experimental.pallas as pl
import jax.experimental.pallas.tpu as pltpu

S, D, H, DH, W, F = 2048, 640, 32, 20, 256, 1728
G = 8
QB = 64
KW = W + QB
BM = 512
NEG = -1e30
QSCALE = (DH ** -0.5) * math.log2(math.e)
P_TILE = tuple((40 * p) // 128 if (40 * p) % 128 <= 88 else 5 + (40 * p - 64) // 128 for p in range(16))
P_OFF = tuple((40 * p) % 128 if (40 * p) % 128 <= 88 else (40 * p - 64) % 128 for p in range(16))


def _pk(v):
    return pltpu.bitcast(v, jnp.uint32)


def _up(v):
    return pltpu.bitcast(v, jnp.bfloat16)


def _ln(x):
    m = jnp.mean(x, axis=-1, keepdims=True)
    xc = x - m
    v = jnp.mean(xc * xc, axis=-1, keepdims=True)
    return xc * lax.rsqrt(v + 1e-5)


def _kernel(x_hbm, wqkv_hbm, wo_hbm, w1_hbm, b1_ref, w2_hbm, b2_ref, out_hbm,
            x_ref, wqkv_ref, wo_ref, w1_ref, w2_ref, obuf, sems,
            xres, qs, ks, vt, ot, wvt, sb0, sb1, pb0, pb1):
    sb = (sb0, sb1)
    pb = (pb0, pb1)
    f32, bf16, u32 = jnp.float32, jnp.bfloat16, jnp.uint32
    NC = S // BM
    x_cp = [pltpu.make_async_copy(x_hbm.at[pl.ds(c_ * BM, BM)], x_ref.at[pl.ds(c_ * BM, BM)], sems.at[c_])
            for c_ in range(NC)]
    w_cp = [pltpu.make_async_copy(h_, v_, sems.at[NC + i_]) for i_, (h_, v_) in enumerate(
        ((wqkv_hbm, wqkv_ref), (wo_hbm, wo_ref), (w1_hbm, w1_ref), (w2_hbm, w2_ref)))]
    w_cp[0].start()
    for cp in x_cp:
        cp.start()
    for cp in w_cp[1:]:
        cp.start()
    qs_b, ks_b, vt_b, ot_b, pb_b = qs, ks, vt, ot, pb
    qs, ks, vt, ot = [r.bitcast(u32) for r in (qs, ks, vt, ot)]
    pb = [r.bitcast(u32) for r in pb]
    vt[0:2] = jnp.zeros((2, 16, 24, 128), u32)
    for r_ in pb:
        r_[...] = jnp.zeros((4, 192, 128), u32)
    w_cp[0].wait()
    wvt[...] = wqkv_ref[:, 2 * D:].astype(f32).T.astype(bf16)

    def out_copy(c):
        return pltpu.make_async_copy(obuf.at[pl.ds(c * BM, BM)], out_hbm.at[pl.ds(c * BM, BM)], sems.at[NC + 4])

    def qkv_chunk(c, first):
        r0 = pl.multiple_of(c * BM, BM)
        if first:
            pltpu.make_async_copy(x_hbm.at[pl.ds(r0, BM)], x_ref.at[pl.ds(r0, BM)], sems.at[c]).wait()
            xc = x_ref[pl.ds(r0, BM), :].astype(f32)
            xres[pl.ds(r0, BM), :] = xc
        else:
            xc = xres[pl.ds(r0, BM), :]
        xb = _ln(xc).astype(bf16)
        q = (jnp.dot(xb, wqkv_ref[:, 0:D], preferred_element_type=f32) * QSCALE).astype(bf16)
        k = jnp.dot(xb, wqkv_ref[:, D:2 * D], preferred_element_type=f32).astype(bf16)
        rh = pl.multiple_of(c * (BM // 2), BM // 2)
        lo64 = lax.broadcasted_iota(jnp.int32, (BM // 2, 128), 1) < 64
        for val, refb, ref, base in ((q, qs_b, qs, 0), (k, ks_b, ks, W)):
            for t in range(5):
                refb[t, pl.ds(base + r0, BM), :] = val[:, 128 * t:128 * (t + 1)]
            rl = [pltpu.roll(ref[t, pl.ds(base // 2 + rh, BM // 2), :], 64, 1) for t in range(5)]
            for t in range(4):
                ref[5 + t, pl.ds(base // 2 + rh, BM // 2), :] = jnp.where(lo64, rl[t], rl[t + 1])
        vTf = lax.dot_general(wvt[...], xb, (((1,), (1,)), ((), ())),
                              preferred_element_type=f32)
        nt = BM // 128
        for t in range(nt):
            for g in range(G):
                v2 = vTf[80 * g:80 * (g + 1), 128 * t:128 * (t + 1)]
                z8 = jnp.ones((8, 128), f32)
                vt_b[2 + c * nt + t, 2 * g] = jnp.concatenate([v2[0:40], z8], axis=0).astype(bf16)
                vt_b[2 + c * nt + t, 2 * g + 1] = jnp.concatenate([v2[40:80], z8], axis=0).astype(bf16)

    lane = lax.broadcasted_iota(jnp.int32, (128, 128), 1)
    row = lax.broadcasted_iota(jnp.int32, (128, 128), 0)
    r32 = lax.broadcasted_iota(jnp.int32, (QB, 128), 0)
    c32 = lax.broadcasted_iota(jnp.int32, (QB, 128), 1) % QB
    orow = lax.broadcasted_iota(jnp.int32, (80, 128), 0) // DH
    olane = lax.broadcasted_iota(jnp.int32, (80, 128), 1) // QB

    r8 = lax.broadcasted_iota(jnp.int32, (8, 128), 0)
    l8 = lax.broadcasted_iota(jnp.int32, (8, 128), 1) // QB

    def stage_a(g, J, s, sref):
        tile = jnp.int32(0)
        off = jnp.int32(0)
        pp, s = s // 2, s % 2
        for gg in range(G):
            tile = jnp.where(g == gg, P_TILE[2 * gg + pp], tile)
            off = jnp.where(g == gg, P_OFF[2 * gg + pp], off)
        lo = off + DH * (row // QB)
        qmask = (lane >= lo) & (lane < lo + DH)
        qh = pl.multiple_of(J * 64 + s * (QB // 2), QB // 2)
        q = _up(qs[tile, pl.ds(qh, QB // 2), :])
        qbd = jnp.where(qmask, jnp.concatenate([q] * (128 // QB), axis=0), jnp.zeros((), bf16))
        kb = _up(ks[tile, pl.ds(qh, KW // 2), :])
        sref[...] = lax.dot_general(kb, qbd, (((1,), (1,)), ((), ())), preferred_element_type=f32)

    def stage_b(sref, pref):
        po = QB * (pref[0] % 2)
        pref = pref[1].at[pref[0]]
        top = jnp.where(r32 > c32, sref[0:QB], NEG)
        bot = jnp.where(r32 <= c32, sref[W:KW], NEG)
        mid = [sref[QB + QB * i:QB + QB * (i + 1)] for i in range(3)]
        parts = [top] + mid + [bot]
        mx = parts[0]
        for t in parts[1:]:
            mx = jnp.maximum(mx, t)
        m = jnp.max(mx, axis=0, keepdims=True)
        for i, t in enumerate(parts):
            pref[po + QB * i:po + QB * (i + 1)] = jnp.exp2(t - m).astype(bf16)

    def stage_c(g, J, s, pref, acc):
        pp, s = s // 2, s % 2
        g = 2 * g + pp
        o = jnp.dot(_up(vt[J, g]), _up(pref[0:64]), preferred_element_type=f32)
        o += jnp.dot(_up(vt[J + 1, g]), _up(pref[64:128]), preferred_element_type=f32)
        o += jnp.dot(_up(vt[J + 2, g])[:, 0:QB * (s + 1)], _up(pref[128:128 + 32 * (s + 1)]), preferred_element_type=f32)
        rl = 1.0 / o[40:48]
        for i in range(5):
            oi = o[8 * i:8 * i + 8] * rl
            for h in sorted({(8 * i) // DH, (8 * i + 7) // DH}):
                sh = (QB * (s - h)) % 128
                oo = oi if sh == 0 else pltpu.roll(oi, sh, 1)
                msk = l8 == s
                if (8 * i) // DH != (8 * i + 7) // DH:
                    msk = msk & ((r8 + 8 * i) // DH == h)
                acc[5 * pp + i] = jnp.where(msk, oo, acc[5 * pp + i])

    def store_o(g, J, acc):
        ot_b[J, pl.ds(pl.multiple_of(g * 80, 16), 80), :] = jnp.concatenate(acc, axis=0).astype(bf16)

    NF = S // 128

    def gj(i):
        i = jnp.minimum(i, G * NF - 1)
        return i // NF, i % NF

    def a_fast(i2, _):
        for par in range(2):
            i = 2 * i2 + par
            g, J = gj(i)
            g2, J2 = gj(i + 2)
            acc = [jnp.zeros((8, 128), f32)] * 10
            for s in range(4):
                stage_b(sb[1 - par].at[s], (s, pb_b[1 - par]))
            for s in range(4):
                stage_c(g, J, s, pb[par].at[s], acc)
            for s in range(4):
                stage_a(g2, J2, s, sb[par].at[s])
            store_o(g, J, acc)
        return 0

    def post_chunk(c, last):
        r0 = pl.multiple_of(c * BM, BM)
        nt = BM // 128
        oT = jnp.concatenate([_up(ot[c * nt + t]) for t in range(nt)], axis=1)
        a = lax.dot_general(oT, wo_ref[...], (((0,), (0,)), ((), ())), preferred_element_type=f32)
        x1 = xres[pl.ds(r0, BM), :] + a
        xb = _ln(x1).astype(bf16)
        hpre = lax.dot_general(xb, w1_ref[...], (((1,), (1,)), ((), ())), preferred_element_type=f32) + b1_ref[...].astype(f32).reshape(1, F)
        hh = jax.nn.gelu(hpre, approximate=True).astype(bf16)
        y = jnp.dot(hh, w2_ref[...], preferred_element_type=f32) + b2_ref[...].astype(f32).reshape(1, D)
        x2 = x1 + y
        if last:
            obuf[pl.ds(r0, BM), :] = x2.astype(obuf.dtype)
            out_copy(c).start()
        else:
            xres[pl.ds(r0, BM), :] = x2

    for layer in range(2):
        def qkv_body(c, _, first=(layer == 0)):
            qkv_chunk(c, first)
            return 0
        with jax.named_scope("qkv"):
            with jax.named_scope("a"):
                lax.fori_loop(0, S // BM, qkv_body, 0)

        with jax.named_scope("attn"):
            for t_ in range(9):
                ks_b[t_, 0:W, :] = jnp.broadcast_to(ks_b[t_, W:W + 16, :][0:1], (W, 128))
            for s_ in range(4):
                stage_a(jnp.int32(0), jnp.int32(0), s_, sb[0].at[s_])
            for s_ in range(4):
                stage_a(jnp.int32(0), jnp.int32(1), s_, sb[1].at[s_])
            for s_ in range(4):
                stage_b(sb[0].at[s_], (s_, pb_b[0]))
            lax.fori_loop(0, G * NF // 2, a_fast, 0)

        if layer == 0:
            for cp in w_cp[1:]:
                cp.wait()

        def post_body(c, _, last=(layer == 1)):
            post_chunk(c, last)
            return 0
        with jax.named_scope("post"):
            lax.fori_loop(0, S // BM, post_body, 0)
    for c_ in range(NC):
        out_copy(c_).wait()


@jax.jit
def pallas_interleave_layers__sliding_block__dense_activation_gelu__prompt_kernel(
        A_x, A_wqkv, A_wo, B_x, B_w1, B_b1, B_w2, B_b2):
    del B_x
    bf16 = jnp.bfloat16
    out = pl.pallas_call(
        _kernel,
        out_shape=jax.ShapeDtypeStruct((S, D), A_x.dtype),
        in_specs=[pl.BlockSpec(memory_space=pl.ANY)] * 4 + [pl.BlockSpec(memory_space=pltpu.VMEM),
                                                             pl.BlockSpec(memory_space=pl.ANY),
                                                             pl.BlockSpec(memory_space=pltpu.VMEM)],
        out_specs=pl.BlockSpec(memory_space=pl.ANY),
        scratch_shapes=[
            pltpu.VMEM((S, D), bf16),
            pltpu.VMEM((D, 3 * D), bf16),
            pltpu.VMEM((D, D), bf16),
            pltpu.VMEM((F, D), bf16),
            pltpu.VMEM((F, D), bf16),
            pltpu.VMEM((S, D), bf16),
            pltpu.SemaphoreType.DMA((S // BM + 5,)),
            pltpu.VMEM((S, D), jnp.float32),
            pltpu.VMEM((9, S, 128), bf16),
            pltpu.VMEM((9, S + W, 128), bf16),
            pltpu.VMEM((18, 16, 48, 128), bf16),
            pltpu.VMEM((16, D, 128), bf16),
            pltpu.VMEM((D, D), bf16),
            pltpu.VMEM((4, KW, 128), jnp.float32),
            pltpu.VMEM((4, KW, 128), jnp.float32),
            pltpu.VMEM((4, 384, 128), bf16),
            pltpu.VMEM((4, 384, 128), bf16),
        ],
        compiler_params=pltpu.CompilerParams(vmem_limit_bytes=100 * 1024 * 1024),
    )(A_x.reshape(S, D), A_wqkv, A_wo, B_w1.T, B_b1, B_w2, B_b2)
    return out.reshape(1, S, D)
```

```python
import math
import jax
import jax.numpy as jnp
from jax import lax
import jax.experimental.pallas as pl
import jax.experimental.pallas.tpu as pltpu

S, D, H, DH, W, F = 2048, 640, 32, 20, 256, 1728
G = 8
QB = 64
KW = W + QB
BM = 512
NEG = -1e30
QSCALE = (DH ** -0.5) * math.log2(math.e)
P_TILE = tuple((40 * p) // 128 if (40 * p) % 128 <= 88 else 5 + (40 * p - 64) // 128 for p in range(16))
P_OFF = tuple((40 * p) % 128 if (40 * p) % 128 <= 88 else (40 * p - 64) % 128 for p in range(16))


def _pk(v):
    return pltpu.bitcast(v, jnp.uint32)


def _up(v):
    return pltpu.bitcast(v, jnp.bfloat16)


def _ln(x):
    m = jnp.mean(x, axis=-1, keepdims=True)
    xc = x - m
    v = jnp.mean(xc * xc, axis=-1, keepdims=True)
    return xc * lax.rsqrt(v + 1e-5)


def _kernel(x_hbm, wqkv_hbm, wo_hbm, w1_hbm, b1_ref, w2_hbm, b2_ref, out_hbm,
            x_ref, wqkv_ref, wo_ref, w1_ref, w2_ref, obuf, sems,
            xres, qs, ks, vt, ot, wvt, sb0, sb1, pb0, pb1):
    sb = (sb0, sb1)
    pb = (pb0, pb1)
    f32, bf16, u32 = jnp.float32, jnp.bfloat16, jnp.uint32
    NC = S // BM
    x_cp = [pltpu.make_async_copy(x_hbm.at[pl.ds(c_ * BM, BM)], x_ref.at[pl.ds(c_ * BM, BM)], sems.at[c_])
            for c_ in range(NC)]
    w_cp = [pltpu.make_async_copy(h_, v_, sems.at[NC + i_]) for i_, (h_, v_) in enumerate(
        ((wqkv_hbm, wqkv_ref), (wo_hbm, wo_ref), (w1_hbm, w1_ref), (w2_hbm, w2_ref)))]
    w_cp[0].start()
    for cp in x_cp:
        cp.start()
    for cp in w_cp[1:]:
        cp.start()
    qs_b, ks_b, vt_b, ot_b, pb_b = qs, ks, vt, ot, pb
    qs, ks, vt, ot = [r.bitcast(u32) for r in (qs, ks, vt, ot)]
    pb = [r.bitcast(u32) for r in pb]
    vt[0:2] = jnp.zeros((2, 16, 24, 128), u32)
    for r_ in pb:
        r_[...] = jnp.zeros((4, 192, 128), u32)
    w_cp[0].wait()
    wvt[...] = wqkv_ref[:, 2 * D:].astype(f32).T.astype(bf16)

    def out_copy(c):
        return pltpu.make_async_copy(obuf.at[pl.ds(c * BM, BM)], out_hbm.at[pl.ds(c * BM, BM)], sems.at[NC + 4])

    def qkv_chunk(c, first):
        r0 = pl.multiple_of(c * BM, BM)
        if first:
            pltpu.make_async_copy(x_hbm.at[pl.ds(r0, BM)], x_ref.at[pl.ds(r0, BM)], sems.at[c]).wait()
            xc = x_ref[pl.ds(r0, BM), :].astype(f32)
            xres[pl.ds(r0, BM), :] = xc
        else:
            xc = xres[pl.ds(r0, BM), :]
        xb = _ln(xc).astype(bf16)
        q = (jnp.dot(xb, wqkv_ref[:, 0:D], preferred_element_type=f32) * QSCALE).astype(bf16)
        k = jnp.dot(xb, wqkv_ref[:, D:2 * D], preferred_element_type=f32).astype(bf16)
        rh = pl.multiple_of(c * (BM // 2), BM // 2)
        lo64 = lax.broadcasted_iota(jnp.int32, (BM // 2, 128), 1) < 64
        for val, refb, ref, base in ((q, qs_b, qs, 0), (k, ks_b, ks, W)):
            for t in range(5):
                refb[t, pl.ds(base + r0, BM), :] = val[:, 128 * t:128 * (t + 1)]
            rl = [pltpu.roll(ref[t, pl.ds(base // 2 + rh, BM // 2), :], 64, 1) for t in range(5)]
            for t in range(4):
                ref[5 + t, pl.ds(base // 2 + rh, BM // 2), :] = jnp.where(lo64, rl[t], rl[t + 1])
        vTf = lax.dot_general(wvt[...], xb, (((1,), (1,)), ((), ())),
                              preferred_element_type=f32)
        nt = BM // 128
        for t in range(nt):
            for g in range(G):
                v2 = vTf[80 * g:80 * (g + 1), 128 * t:128 * (t + 1)]
                z8 = jnp.ones((8, 128), f32)
                vt_b[2 + c * nt + t, 2 * g] = jnp.concatenate([v2[0:40], z8], axis=0).astype(bf16)
                vt_b[2 + c * nt + t, 2 * g + 1] = jnp.concatenate([v2[40:80], z8], axis=0).astype(bf16)

    lane = lax.broadcasted_iota(jnp.int32, (128, 128), 1)
    row = lax.broadcasted_iota(jnp.int32, (128, 128), 0)
    r32 = lax.broadcasted_iota(jnp.int32, (QB, 128), 0)
    c32 = lax.broadcasted_iota(jnp.int32, (QB, 128), 1) % QB

    r8 = lax.broadcasted_iota(jnp.int32, (8, 128), 0)
    l8 = lax.broadcasted_iota(jnp.int32, (8, 128), 1) // QB

    def stage_a(g, J, s, sref):
        tile = jnp.int32(0)
        off = jnp.int32(0)
        pp, s = s // 2, s % 2
        for gg in range(G):
            tile = jnp.where(g == gg, P_TILE[2 * gg + pp], tile)
            off = jnp.where(g == gg, P_OFF[2 * gg + pp], off)
        lo = off + DH * (row // QB)
        qmask = (lane >= lo) & (lane < lo + DH)
        qh = pl.multiple_of(J * 64 + s * (QB // 2), QB // 2)
        q = _up(qs[tile, pl.ds(qh, QB // 2), :])
        qbd = jnp.where(qmask, jnp.concatenate([q] * (128 // QB), axis=0), jnp.zeros((), bf16))
        kb = _up(ks[tile, pl.ds(qh, KW // 2), :])
        sref[...] = lax.dot_general(kb, qbd, (((1,), (1,)), ((), ())), preferred_element_type=f32)

    def stage_b(sref, pref):
        po = QB * (pref[0] % 2)
        pref = pref[1].at[pref[0]]
        top = jnp.where(r32 > c32, sref[0:QB], NEG)
        bot = jnp.where(r32 <= c32, sref[W:KW], NEG)
        mid = [sref[QB + QB * i:QB + QB * (i + 1)] for i in range(3)]
        parts = [top] + mid + [bot]
        mx = parts[0]
        for t in parts[1:]:
            mx = jnp.maximum(mx, t)
        m = jnp.max(mx, axis=0, keepdims=True)
        for i, t in enumerate(parts):
            pref[po + QB * i:po + QB * (i + 1)] = jnp.exp2(t - m).astype(bf16)

    def stage_c(g, J, s, pref, acc):
        pp, s = s // 2, s % 2
        g = 2 * g + pp
        o = jnp.dot(_up(vt[J, g]), _up(pref[0:64]), preferred_element_type=f32)
        o += jnp.dot(_up(vt[J + 1, g]), _up(pref[64:128]), preferred_element_type=f32)
        o += jnp.dot(_up(vt[J + 2, g])[:, 0:QB * (s + 1)], _up(pref[128:128 + 32 * (s + 1)]), preferred_element_type=f32)
        rl = 1.0 / o[40:48]
        for i in range(5):
            oi = o[8 * i:8 * i + 8] * rl
            for h in sorted({(8 * i) // DH, (8 * i + 7) // DH}):
                sh = (QB * (s - h)) % 128
                oo = oi if sh == 0 else pltpu.roll(oi, sh, 1)
                msk = l8 == s
                if (8 * i) // DH != (8 * i + 7) // DH:
                    msk = msk & ((r8 + 8 * i) // DH == h)
                acc[5 * pp + i] = jnp.where(msk, oo, acc[5 * pp + i])

    def store_o(g, J, acc):
        ot_b[J, pl.ds(pl.multiple_of(g * 80, 16), 80), :] = jnp.concatenate(acc, axis=0).astype(bf16)

    NF = S // 128

    def gj(i):
        i = jnp.minimum(i, G * NF - 1)
        return i // NF, i % NF

    def a_fast(i2, _):
        for par in range(2):
            i = 2 * i2 + par
            g, J = gj(i)
            g2, J2 = gj(i + 2)
            acc = [jnp.zeros((8, 128), f32)] * 10
            for s in range(4):
                stage_b(sb[1 - par].at[s], (s, pb_b[1 - par]))
            for s in range(4):
                stage_c(g, J, s, pb[par].at[s], acc)
            for s in range(4):
                stage_a(g2, J2, s, sb[par].at[s])
            store_o(g, J, acc)
        return 0

    def post_chunk(c, last):
        r0 = pl.multiple_of(c * BM, BM)
        nt = BM // 128
        oT = jnp.concatenate([_up(ot[c * nt + t]) for t in range(nt)], axis=1)
        a = lax.dot_general(oT, wo_ref[...], (((0,), (0,)), ((), ())), preferred_element_type=f32)
        x1 = xres[pl.ds(r0, BM), :] + a
        xb = _ln(x1).astype(bf16)
        hpre = lax.dot_general(xb, w1_ref[...], (((1,), (1,)), ((), ())), preferred_element_type=f32) + b1_ref[...].astype(f32).reshape(1, F)
        hh = jax.nn.gelu(hpre, approximate=True).astype(bf16)
        y = jnp.dot(hh, w2_ref[...], preferred_element_type=f32) + b2_ref[...].astype(f32).reshape(1, D)
        x2 = x1 + y
        if last:
            obuf[pl.ds(r0, BM), :] = x2.astype(obuf.dtype)
            out_copy(c).start()
        else:
            xres[pl.ds(r0, BM), :] = x2

    for layer in range(2):
        def qkv_body(c, _, first=(layer == 0)):
            qkv_chunk(c, first)
            return 0
        with jax.named_scope("qkv"):
            lax.fori_loop(0, S // BM, qkv_body, 0)

        with jax.named_scope("attn"):
            for t_ in range(9):
                ks_b[t_, 0:W, :] = jnp.broadcast_to(ks_b[t_, W:W + 16, :][0:1], (W, 128))
            for s_ in range(4):
                stage_a(jnp.int32(0), jnp.int32(0), s_, sb[0].at[s_])
            for s_ in range(4):
                stage_a(jnp.int32(0), jnp.int32(1), s_, sb[1].at[s_])
            for s_ in range(4):
                stage_b(sb[0].at[s_], (s_, pb_b[0]))
            lax.fori_loop(0, G * NF // 2, a_fast, 0)

        if layer == 0:
            for cp in w_cp[1:]:
                cp.wait()

        def post_body(c, _, last=(layer == 1)):
            post_chunk(c, last)
            return 0
        with jax.named_scope("post"):
            lax.fori_loop(0, S // BM, post_body, 0)
    for c_ in range(NC):
        out_copy(c_).wait()


@jax.jit
def pallas_interleave_layers__sliding_block__dense_activation_gelu__prompt_kernel(
        A_x, A_wqkv, A_wo, B_x, B_w1, B_b1, B_w2, B_b2):
    del B_x
    bf16 = jnp.bfloat16
    out = pl.pallas_call(
        _kernel,
        out_shape=jax.ShapeDtypeStruct((S, D), A_x.dtype),
        in_specs=[pl.BlockSpec(memory_space=pl.ANY)] * 4 + [pl.BlockSpec(memory_space=pltpu.VMEM),
                                                             pl.BlockSpec(memory_space=pl.ANY),
                                                             pl.BlockSpec(memory_space=pltpu.VMEM)],
        out_specs=pl.BlockSpec(memory_space=pl.ANY),
        scratch_shapes=[
            pltpu.VMEM((S, D), bf16),
            pltpu.VMEM((D, 3 * D), bf16),
            pltpu.VMEM((D, D), bf16),
            pltpu.VMEM((F, D), bf16),
            pltpu.VMEM((F, D), bf16),
            pltpu.VMEM((S, D), bf16),
            pltpu.SemaphoreType.DMA((S // BM + 5,)),
            pltpu.VMEM((S, D), jnp.float32),
            pltpu.VMEM((9, S, 128), bf16),
            pltpu.VMEM((9, S + W, 128), bf16),
            pltpu.VMEM((18, 16, 48, 128), bf16),
            pltpu.VMEM((16, D, 128), bf16),
            pltpu.VMEM((D, D), bf16),
            pltpu.VMEM((4, KW, 128), jnp.float32),
            pltpu.VMEM((4, KW, 128), jnp.float32),
            pltpu.VMEM((4, 384, 128), bf16),
            pltpu.VMEM((4, 384, 128), bf16),
        ],
        compiler_params=pltpu.CompilerParams(vmem_limit_bytes=100 * 1024 * 1024),
    )(A_x.reshape(S, D), A_wqkv, A_wo, B_w1.T, B_b1, B_w2, B_b2)
    return out.reshape(1, S, D)
```
